```python
import os as _os
_os.environ.setdefault("JAX_PLATFORMS", "cpu")
import jax
import jax.numpy as jnp

def _softmax(x, axis=-1):
    return jax.nn.softmax(x, axis=axis)
def _gelu(x):
    return jax.nn.gelu(x, approximate=True)
def _silu(x):
    return jax.nn.silu(x)
def _sigmoid(x):
    return jax.nn.sigmoid(x)
def _layernorm(x, axis=-1, eps=1e-5):
    m = jnp.mean(x, axis=axis, keepdims=True)
    v = jnp.var(x, axis=axis, keepdims=True)
    return (x - m) / jnp.sqrt(v + eps)
def _scatter_add(tgt, idx, src, axis=0):
    return tgt.at[idx].add(src)
def _segment_sum(src, seg, n):
    return jax.ops.segment_sum(src, seg, n)
class _Rng:
    def __init__(self, key):
        self._k = key
    def _next(self):
        self._k, sub = jax.random.split(self._k)
        return sub
    def normal(self, shape):
        return jax.random.normal(self._next(), shape, dtype=jnp.bfloat16)
    def randint(self, lo, hi, shape):
        return jax.random.randint(self._next(), shape, lo, hi, dtype=jnp.int32)
    def uniform(self, shape, lo=0.0, hi=1.0):
        return jax.random.uniform(self._next(), shape, jnp.bfloat16, lo, hi)
    def permutation(self, n):
        return jax.random.permutation(self._next(), n)


kernel_name = 'concat_heads__gqa_block_cached__mha_block_cached__near_ridge'

def setup_inputs():
    _rng = _Rng(jax.random.key(int.from_bytes(__import__("os").urandom(4), "little")))
    _w = (lambda a: (lambda t: t.astype(jnp.bfloat16) if jnp.issubdtype(t.dtype, jnp.floating) else t)(jnp.asarray(a)))
    def _A_setup():
        B, Sq, D = 16, 32, 1024
        Hq, Hkv, Sk, Dh = 32, 4, 32, 128
        assert Hq % Hkv == 0, (Hq, Hkv)
        return {
            "x": _w((lambda *s: _rng.normal(s) * 0.8)(B, Sq, D)),
            "k_cache": _w((lambda *s: _rng.normal(s) * 0.8)(B, Hkv, Sk, Dh)),
            "v_cache": _w((lambda *s: _rng.normal(s) * 0.05)(B, Hkv, Sk, Dh)),
            "wq": _w((lambda *s: _rng.normal(s) * 0.8)(D, Hq * Dh) * (D ** -0.5)),
            "wo": _w((lambda *s: _rng.normal(s) * 0.05)(Hq * Dh, D) * ((Hq * Dh) ** -0.5)),
        }
    _A_in = _A_setup()

    def _B_setup():
        B, Sq, D = 16, 32, 1024
        H, Sk, Dh = 32, 32, 128
        return {
            "x": _w((lambda *s: _rng.normal(s) * 0.8)(B, Sq, D)),
            "k_cache": _w((lambda *s: _rng.normal(s) * 0.8)(B, H, Sk, Dh)),
            "v_cache": _w((lambda *s: _rng.normal(s) * 0.05)(B, H, Sk, Dh)),
            "wq": _w((lambda *s: _rng.normal(s) * 0.8)(D, H * Dh) * (D ** -0.5)),
            "wo": _w((lambda *s: _rng.normal(s) * 0.05)(H * Dh, D) * ((H * Dh) ** -0.5)),
        }
    _B_in = _B_setup()

    return {
        "A_x": _A_in["x"],
        "A_k_cache": _A_in["k_cache"],
        "A_v_cache": _A_in["v_cache"],
        "A_wq": _A_in["wq"],
        "A_wo": _A_in["wo"],
        "B_x": _B_in["x"],
        "B_k_cache": _B_in["k_cache"],
        "B_v_cache": _B_in["v_cache"],
        "B_wq": _B_in["wq"],
        "B_wo": _B_in["wo"],
    }

def reference(A_x, A_k_cache, A_v_cache, A_wq, A_wo, B_x, B_k_cache, B_v_cache, B_wq, B_wo):
    def _A_ref(x, k_cache, v_cache, wq, wo):
        B, Sq, D = x.shape
        Hq, Dh = 32, 128
        Hkv = k_cache.shape[1]
        rep = Hq // Hkv
        q = (lambda x, *d: x.transpose(*d))((x @ wq).reshape(B, Sq, Hq, Dh), 0, 2, 1, 3)
        k = jnp.repeat(k_cache, rep, axis=1)
        v = jnp.repeat(v_cache, rep, axis=1)
        scores = jnp.einsum("bhqd,bhkd->bhqk", q, k) * (Dh ** -0.5)
        p = _softmax(scores, axis=-1)
        o = jnp.einsum("bhqk,bhkd->bhqd", p, v)
        return (lambda x, *d: x.transpose(*d))(o, 0, 2, 1, 3).reshape(B, Sq, Hq * Dh) @ wo

    def _B_ref(x, k_cache, v_cache, wq, wo):
        B, Sq, D = x.shape
        H, Dh = 32, 128
        q = (lambda x, *d: x.transpose(*d))((x @ wq).reshape(B, Sq, H, Dh), 0, 2, 1, 3)
        scores = jnp.einsum("bhqd,bhkd->bhqk", q, k_cache) * (Dh ** -0.5)
        p = _softmax(scores, axis=-1)
        o = jnp.einsum("bhqk,bhkd->bhqd", p, v_cache)
        return (lambda x, *d: x.transpose(*d))(o, 0, 2, 1, 3).reshape(B, Sq, H * Dh) @ wo

    a = _A_ref(A_x, A_k_cache, A_v_cache, A_wq, A_wo)
    b = _B_ref(B_x, B_k_cache, B_v_cache, B_wq, B_wo)
    return jnp.concatenate([a, b], axis=-1)
```

```python
import os
import functools
import math
import jax
import jax.numpy as jnp
import jax.experimental.pallas as pl
import jax.experimental.pallas.tpu as pltpu

U = 2
POLICY = os.environ.get('KW_POLICY', 'staged')
B, SQ, D, H, SK, DH = 16, 32, 1024, 32, 32, 128
M = B * SQ
SCALE = DH ** -0.5
C2 = SCALE * math.log2(math.e)
NT = (((1,), (1,)), ((), ()))
NUB = H // U
NU = 2 * NUB
UW = U * DH
f32 = jnp.float32
bf = jnp.bfloat16

STEPS = [('Q', 0, 0), ('Q', 0, 1)]
for u in range(NU):
    STEPS.append(('QK', u))
    if u + 1 < NU:
        STEPS.append(('Q', u + 1, None))
    else:
        STEPS.append(('O', u - 1))
    STEPS.append(('PV', u))
    if 1 <= u < NU - 1:
        STEPS.append(('O', u - 1))
STEPS.append(('O', NU - 1))

GROUPS = [
    (('Q', 0, 0), [('x', 0, 0, 256), ('wq', 0, 0, 1)]),
    (('Q', 0, 1), [('x', 0, 256, 512)]),
    (('QK', 0), [('wq', 0, 1, 2), ('k', 0, 0, 1)]),
    (('PV', 0), [('v', 0, 0, 1), ('wq', 0, 2, 3), ('wo', 0, 0, 1)]),
    (('QK', 2), [('wq', 0, 3, 5), ('wo', 0, 1, 3)]),
    (('QK', 4), [('k', 0, 1, 4), ('v', 0, 1, 4), ('wq', 0, 5, 9), ('wo', 0, 3, 7)]),
    (('QK', 8), [('wq', 0, 9, 16), ('wo', 0, 7, 14)]),
    (('QK', 15), [('wo', 0, 14, 16), ('x', 1, 0, 512), ('wq', 1, 0, 11), ('k', 1, 0, 20), ('v', 1, 0, 20), ('wo', 1, 0, 9)]),
    (('QK', 26), [('wq', 1, 11, 16), ('k', 1, 20, 32), ('v', 1, 20, 32), ('wo', 1, 9, 16)]),
]
NSEM = sum(len(g[1]) for g in GROUPS)


def _kernel(xa_h, ka_h, va_h, wqa_h, woa_h, xb_h, kb_h, vb_h, wqb_h, wob_h, out_h,
            x_v, ka_v, va_v, kb_v, vb_v, wq_v, wo_v, acc, q0, q1, o0, o1, outb,
            sems, sem_out):
    qs = (q0, q1)
    os_ = (o0, o1)
    row = jax.lax.broadcasted_iota(jnp.int32, (128, 128), 0) // 32
    col = jax.lax.broadcasted_iota(jnp.int32, (128, 128), 1) // 32
    mask = row == col

    def mk(item, sem):
        kind, r, lo, hi = item
        if kind == 'x':
            return pltpu.make_async_copy((xa_h, xb_h)[r].at[lo:hi], x_v.at[r, lo:hi], sem)
        if kind == 'wq':
            return pltpu.make_async_copy((wqa_h, wqb_h)[r].at[:, lo * UW:hi * UW],
                                         wq_v.at[r, :, lo * UW:hi * UW], sem)
        if kind == 'wo':
            return pltpu.make_async_copy((woa_h, wob_h)[r].at[lo * UW:hi * UW],
                                         wo_v.at[r, lo * UW:hi * UW], sem)
        if kind == 'k':
            return pltpu.make_async_copy((ka_h, kb_h)[r].at[:, lo:hi], (ka_v, kb_v)[r].at[:, lo:hi], sem)
        if kind == 'v':
            return pltpu.make_async_copy((va_h, vb_h)[r].at[:, lo:hi], (va_v, vb_v)[r].at[:, lo:hi], sem)

    gcopies = []
    si = 0
    for at, items in GROUPS:
        cps = []
        for it in items:
            cps.append(mk(it, sems.at[si]))
            si += 1
        gcopies.append(cps)

    def cp_out(r):
        return pltpu.make_async_copy(outb.at[r], out_h.at[:, pl.ds(r * D, D)], sem_out.at[r])

    def qproj(u, part):
        r, c = divmod(u, NUB)
        lo, hi = (0, M) if part is None else (part * 256, part * 256 + 256)
        qs[u % 2][lo:hi] = jnp.dot(x_v[r, lo:hi], wq_v[r, :, c * UW:(c + 1) * UW],
                                   preferred_element_type=f32).astype(bf)

    def kv(ref_a, ref_b, u, hh, bg):
        r, c = divmod(u, NUB)
        h = c * U + hh
        if r == 0:
            return ref_a[bg * 4:(bg + 1) * 4, h // 8].reshape(128, 128)
        return ref_b[bg * 4:(bg + 1) * 4, h].reshape(128, 128)

    def qk(u):
        res = []
        for hh in range(U):
            for bg in range(4):
                q4 = qs[u % 2][bg * 128:(bg + 1) * 128, hh * 128:(hh + 1) * 128]
                s = jax.lax.dot_general(q4, kv(ka_v, kb_v, u, hh, bg), NT, preferred_element_type=f32)
                s = jnp.where(mask, s, -jnp.inf)
                m = jnp.max(s, axis=-1, keepdims=True)
                e = jnp.exp2((s - m) * C2)
                l = jnp.sum(e, axis=-1, keepdims=True)
                res.append((e.astype(bf), pl.reciprocal(l, approx=True)))
        return res

    def pv(u, res):
        i = 0
        for hh in range(U):
            for bg in range(4):
                e, rl = res[i]
                i += 1
                o = jnp.dot(e, kv(va_v, vb_v, u, hh, bg), preferred_element_type=f32) * rl
                os_[u % 2][bg * 128:(bg + 1) * 128, hh * 128:(hh + 1) * 128] = o.astype(bf)

    def oproj(u):
        r, c = divmod(u, NUB)
        res = jnp.dot(os_[u % 2][...], wo_v[r, c * UW:(c + 1) * UW, :], preferred_element_type=f32)
        if c == 0:
            acc[...] = res
        elif c == NUB - 1:
            outb[r] = (acc[...] + res).astype(bf)
            cp_out(r).start()
        else:
            acc[...] += res

    NG = len(GROUPS)
    if POLICY == 'upfront':
        lead = NG
    else:
        lead = int(POLICY[-1]) if POLICY[-1].isdigit() else 2
    for g in range(min(lead, NG)):
        for cp in gcopies[g]:
            cp.start()
    wait_at = {at: g for g, (at, _) in enumerate(GROUPS)}
    pend = {}
    for st in STEPS:
        if st in wait_at:
            g = wait_at[st]
            for cp in gcopies[g]:
                cp.wait()
            if g + lead < NG:
                for cp in gcopies[g + lead]:
                    cp.start()
        if st[0] == 'Q':
            qproj(st[1], st[2])
        elif st[0] == 'QK':
            pend[st[1]] = qk(st[1])
        elif st[0] == 'PV':
            pv(st[1], pend.pop(st[1]))
        else:
            oproj(st[1])
    cp_out(0).wait()
    cp_out(1).wait()


@jax.jit
def pallas_concat_heads__gqa_block_cached__mha_block_cached__near_ridge_kernel(
    A_x, A_k_cache, A_v_cache, A_wq, A_wo, B_x, B_k_cache, B_v_cache, B_wq, B_wo):
    xa = A_x.reshape(M, D)
    xb = B_x.reshape(M, D)
    out = pl.pallas_call(
        _kernel,
        in_specs=[pl.BlockSpec(memory_space=pl.ANY)] * 10,
        out_specs=pl.BlockSpec(memory_space=pl.ANY),
        out_shape=jax.ShapeDtypeStruct((M, 2 * D), bf),
        scratch_shapes=[
            pltpu.VMEM((2, M, D), bf),
            pltpu.VMEM((B, 4, SK, DH), bf), pltpu.VMEM((B, 4, SK, DH), bf),
            pltpu.VMEM((B, H, SK, DH), bf), pltpu.VMEM((B, H, SK, DH), bf),
            pltpu.VMEM((2, D, H * DH), bf), pltpu.VMEM((2, H * DH, D), bf),
            pltpu.VMEM((M, D), f32),
            pltpu.VMEM((M, UW), bf), pltpu.VMEM((M, UW), bf),
            pltpu.VMEM((M, UW), bf), pltpu.VMEM((M, UW), bf),
            pltpu.VMEM((2, M, D), bf),
            pltpu.SemaphoreType.DMA((NSEM,)),
            pltpu.SemaphoreType.DMA((2,)),
        ],
        compiler_params=pltpu.CompilerParams(vmem_limit_bytes=100 * 1024 * 1024),
    )(xa, A_k_cache, A_v_cache, A_wq, A_wo, xb, B_k_cache, B_v_cache, B_wq, B_wo)
    return out.reshape(B, SQ, 2 * D)
```

```python
import math

import jax
import jax.numpy as jnp
import jax.experimental.pallas as pl
import jax.experimental.pallas.tpu as pltpu

B, SQ, D, H, SK, DH = 16, 32, 1024, 32, 32, 128
HKV = 4
M = B * SQ
C2 = DH ** -0.5 * math.log2(math.e)
NT = (((1,), (1,)), ((), ()))
U = 2
NUB = H // U
NU = 2 * NUB
UW = U * DH
PAD = 128
f32 = jnp.float32
bf = jnp.bfloat16
NA_IT = 3
LB = 5
NB_IT = 3
NSLOT = 5
NP1 = 4
KST = (1, 1, 2, 3, 1)
RA = 256

GROUPS = []
_k0 = 0
for _n in KST:
    GROUPS.append([('xk', _k0, _k0 + _n * 128), ('wqk', _k0, _k0 + _n * 128)])
    _k0 += _n * 128
GROUPS[-1] += [('ka', 0, 1), ('wq', 4, 5), ('va', 0, 1)]
G_P2 = len(GROUPS)
GROUPS.append([('wo', 0, 3)])
G_A0 = len(GROUPS)
for _i in range(NA_IT):
    _u0 = 4 + 4 * _i
    GROUPS.append([('wq', _u0 + 1, _u0 + 5), ('wo', _u0 - 1, _u0 + 3),
                   ('ka', 1 + _i, 2 + _i), ('va', 1 + _i, 2 + _i)])
G_B0 = len(GROUPS)
for _i in range(NB_IT):
    _u0 = NUB + _i * LB
    _h0 = (_u0 - NUB) * U
    GROUPS.append([('kb', _h0, _h0 + LB * U), ('wo', _u0 - 1, _u0 - 1 + LB),
                   ('wq', _u0 + 1, _u0 + 1 + LB), ('vb', _h0, _h0 + LB * U)])
G_E = len(GROUPS)
GROUPS.append([('kb', H - U, H), ('vb', H - U, H), ('wo', NU - 2, NU)])
NG = len(GROUPS)
EXTRA = {G_A0 + NA_IT - 1: [('xb', 0, M)]}


def _split(lo, hi, n):
    res = []
    while lo < hi:
        r = lo // n
        e = min(hi, (r + 1) * n)
        res.append((r, lo - r * n, e - r * n, lo, e))
        lo = e
    return res


def _kernel(xa_h, ka_h, va_h, wqa_h, woa_h, xb_h, kb_h, vb_h, wqb_h, wob_h, out_h,
            x_v, ka_v, va_v, kb_v, vb_v, wq_v, wo_v, acc, qacc, outa, outb, sems, sem_out, cnt, *slots):
    qs = slots[:NSLOT]
    os_ = slots[NSLOT:]

    def mk(item, sem):
        kind, lo, hi = item
        if kind == 'xk':
            return [pltpu.make_async_copy(xa_h.at[:, lo:hi], x_v.at[0:M, lo:hi], sem)]
        if kind == 'wqk':
            return [pltpu.make_async_copy(wqa_h.at[lo:hi, 0:NP1 * UW], wq_v.at[lo:hi, 0:NP1 * UW], sem)]
        if kind == 'xb':
            return [pltpu.make_async_copy(xb_h, x_v.at[M:2 * M, 0:D], sem)]
        if kind == 'wq':
            return [pltpu.make_async_copy((wqa_h, wqb_h)[r].at[:, a * UW:b * UW],
                                          wq_v.at[:, ga * UW:gb * UW], sem)
                    for r, a, b, ga, gb in _split(lo, hi, NUB)]
        if kind == 'wo':
            return [pltpu.make_async_copy((woa_h, wob_h)[r].at[a * UW:b * UW],
                                          wo_v.at[ga * UW:gb * UW, 0:D], sem)
                    for r, a, b, ga, gb in _split(lo, hi, NUB)]
        src, dst = {'ka': (ka_h, ka_v), 'va': (va_h, va_v), 'kb': (kb_h, kb_v), 'vb': (vb_h, vb_v)}[kind]
        return [pltpu.make_async_copy(src.at[:, lo:hi], dst.at[:, lo:hi], sem)]

    def copies(items, sem):
        cps = []
        for it in items:
            cps += mk(it, sem)
        return cps

    def wait_items(items, sem):
        for cp in copies(items, sem):
            cp.wait()

    def wait_group(g, gdyn=None):
        wait_items(GROUPS[g], sems.at[g if gdyn is None else gdyn])

    def body_all():
        row = jax.lax.broadcasted_iota(jnp.int32, (128, 128), 0) // 32
        col = jax.lax.broadcasted_iota(jnp.int32, (128, 128), 1) // 32
        mask = row == col

        def recip(l):
            r = pl.reciprocal(l, approx=True)
            return r * (2.0 - l * r)

        def off(u, n):
            if isinstance(u, int):
                return u * n
            return pl.multiple_of(u * n, n)

        def qproj(u, slot, hh=None):
            xs = x_v[pl.ds(off(u // NUB, M), M), 0:D]
            if hh is None:
                qs[slot][...] = jnp.dot(xs, wq_v[:, pl.ds(off(u, UW), UW)],
                                        preferred_element_type=f32).astype(bf)
            else:
                qs[slot][:, hh * DH:(hh + 1) * DH] = jnp.dot(
                    xs, wq_v[:, pl.ds(off(u * U + hh, DH), DH)], preferred_element_type=f32).astype(bf)

        def qk(u, slot):
            res = []
            for hh in range(U):
                for bg in range(4):
                    q4 = qs[slot][bg * 128:(bg + 1) * 128, hh * 128:(hh + 1) * 128]
                    k4 = kb_v[bg * 4:(bg + 1) * 4, (u - NUB) * U + hh].reshape(128, 128)
                    s = jax.lax.dot_general(q4, k4, NT, preferred_element_type=f32)
                    s = jnp.where(mask, s, -jnp.inf)
                    m = jnp.max(s, axis=-1, keepdims=True)
                    e = jnp.exp2((s - m) * C2)
                    l = jnp.sum(e, axis=-1, keepdims=True)
                    res.append((e.astype(bf), recip(l)))
            return res

        def pv(u, slot, res):
            i = 0
            for hh in range(U):
                for bg in range(4):
                    e, rl = res[i]
                    i += 1
                    v4 = vb_v[bg * 4:(bg + 1) * 4, (u - NUB) * U + hh].reshape(128, 128)
                    o = jnp.dot(e, v4, preferred_element_type=f32) * rl
                    os_[slot][bg * 128:(bg + 1) * 128, hh * 128:(hh + 1) * 128] = o.astype(bf)

        def qk_a(v, sl, bg):
            g = v // 2
            ps = []
            for j in range(4):
                b = bg * 4 + j
                w = jnp.concatenate([qs[sl[h // 2]][b * 32:(b + 1) * 32, (h % 2) * 128:(h % 2 + 1) * 128]
                                     for h in range(4)], axis=0)
                st = jax.lax.dot_general(ka_v[b, g], w, NT, preferred_element_type=f32)
                m = jnp.max(st, axis=0, keepdims=True)
                e = jnp.exp2((st - m) * C2)
                l = jnp.sum(e, axis=0, keepdims=True)
                ps.append(e * recip(l))
            return jnp.concatenate(ps, axis=0).T

        def pv_a(v, sl, ts):
            g = v // 2
            for bg in range(4):
                lhs = jnp.concatenate([jnp.where(col == j, ts[bg], 0.0).astype(bf) for j in range(4)],
                                      axis=0)
                w = va_v[bg * 4:(bg + 1) * 4, g].reshape(128, 128)
                o = jnp.dot(lhs, w, preferred_element_type=f32).astype(bf)
                for j in range(4):
                    b = bg * 4 + j
                    for h in range(4):
                        os_[sl[h // 2]][b * 32:(b + 1) * 32, (h % 2) * 128:(h % 2 + 1) * 128] = \
                            o[j * 128 + h * 32:j * 128 + (h + 1) * 32]

        def oproj(u, sl, lo=0, hi=M, c0=0, c1=D):
            n = len(sl)
            if n == 1:
                lhs = os_[sl[0]][lo:hi]
            else:
                lhs = jnp.concatenate([os_[s][lo:hi] for s in sl], axis=1)
            return jnp.dot(lhs, wo_v[pl.ds(off(u, UW), n * UW), c0:c1], preferred_element_type=f32)

        def round_a(v, s0):
            qproj(2 * v + 1, s0 + 1)
            ts = []
            for bg in range(4):
                c0, c1 = bg * 256, (bg + 1) * 256
                acc[0, :, c0:c1] += oproj(2 * v - 1, [s0], c0=c0, c1=c1)
                ts.append(qk_a(v, [s0, s0 + 1], bg))
            qproj(2 * v + 2, (s0 + 2) % 4, hh=0)
            pv_a(v, [s0 + 1, (s0 + 2) % 4], ts)
            qproj(2 * v + 2, (s0 + 2) % 4, hh=1)
            acc[0] += oproj(2 * v, [s0 + 1])

        def round_b(u, j):
            r = (u - 1) // NUB
            if j == 0:
                acc[r, :, 0:256] += oproj(u - 1, [j], c0=0, c1=256)
                res = qk(u, j)
                acc[r, :, 256:D] += oproj(u - 1, [j], c0=256, c1=D)
            else:
                res = qk(u, j)
                acc[r] += oproj(u - 1, [j])
            qproj(u + 1, (j + 1) % LB)
            pv(u, (j + 1) % LB, res)

        def cp_out_b(lo, hi, c0, c1):
            return pltpu.make_async_copy(outb.at[lo:hi, c0:c1], out_h.at[lo:hi, D + c0:D + c1],
                                         sem_out.at[0])

        def cp_out_a(i):
            return pltpu.make_async_copy(outa.at[pl.ds(off(i, RA), RA)],
                                         out_h.at[pl.ds(off(i, RA), RA), pl.ds(0, D)], sem_out.at[0])

        for g in range(NG):
            for cp in copies(EXTRA.get(g, []) + GROUPS[g], sems.at[g]):
                cp.start()
        acc[...] = jnp.zeros_like(acc)

        kk = 0
        for g, n in enumerate(KST[:-1]):
            wait_group(g)
            part = jnp.dot(x_v[0:M, kk:kk + n * 128], wq_v[kk:kk + n * 128, 0:NP1 * UW],
                           preferred_element_type=f32)
            if g == 0:
                qacc[...] = part
            else:
                qacc[...] += part
            kk += n * 128
        wait_group(len(KST) - 1)

        def qfin(u0, u1):
            c0, c1 = u0 * UW, u1 * UW
            part = jnp.dot(x_v[0:M, kk:D], wq_v[kk:D, c0:c1], preferred_element_type=f32)
            res = (qacc[:, c0:c1] + part).astype(bf)
            for u in range(u0, u1):
                qs[u][...] = res[:, (u - u0) * UW:(u - u0 + 1) * UW]

        qfin(0, 2)
        qfin(2, 4)
        ts = [qk_a(0, [0, 1], bg) for bg in range(4)]
        qproj(4, 0, 0)
        pv_a(0, [1, 2], ts)
        wait_group(G_P2)
        ts = []
        for bg in range(4):
            c0, c1 = bg * 256, (bg + 1) * 256
            acc[0, :, c0:c1] += oproj(0, [1], c0=c0, c1=c1)
            ts.append(qk_a(1, [2, 3], bg))
        qproj(4, 0, 1)
        pv_a(1, [3, 0], ts)
        acc[0] += oproj(1, [2, 3])

        def a_body(i, carry):
            for g, items in EXTRA.items():
                @pl.when(i == g - G_A0)
                def _():
                    wait_items(items, sems.at[g])
            wait_group(G_A0, G_A0 + i)
            round_a(2 + 2 * i, 0)
            round_a(3 + 2 * i, 2)
            return carry
        jax.lax.fori_loop(0, NA_IT, a_body, 0)

        def b_body(i, carry):
            wait_group(G_B0 + 1, G_B0 + i)
            for j in range(LB):
                round_b(NUB + i * LB + j, j)
                if j == 0:
                    src = jnp.minimum(i, M // RA - 1)
                    outa[pl.ds(off(i, RA), RA), :] = acc[0, pl.ds(off(src, RA), RA), :].astype(bf)

                    @pl.when(i < M // RA)
                    def _():
                        cp_out_a(src).start()
            return carry
        jax.lax.fori_loop(0, NB_IT, b_body, 0)

        wait_group(G_E)
        u = NU - 1
        acc[1, 192:256] += oproj(u - 1, [0], 192, 256)
        res = qk(u, 0)
        acc[1, 256:512] += oproj(u - 1, [0], 256, 512)
        pv(u, 1, res)
        acc[1, 128:192] += oproj(u - 1, [0], 128, 192)
        pieces = [(256, 384, 1, 0, D), (384, 512, 1, 0, D), (128, 256, 1, 0, D)]
        pieces += [(0, 128, 2, c * 128, (c + 1) * 128) for c in range(D // 128)]
        for lo, hi, n, c0, c1 in pieces:
            last = oproj(u - 1, [0, 1], lo, hi, c0, c1) if n == 2 else oproj(u, [1], lo, hi, c0, c1)
            outb[lo:hi, c0:c1] = (acc[1, lo:hi, c0:c1] + last).astype(bf)
            cp_out_b(lo, hi, c0, c1).start()
        for i in range(M // RA):
            cp_out_a(i).wait()
        for lo, hi, n, c0, c1 in pieces:
            cp_out_b(lo, hi, c0, c1).wait()

    cnt[0] = 1

    def outer(i, carry):
        body_all()
        return carry
    jax.lax.fori_loop(0, cnt[0], outer, 0)


@jax.jit
def pallas_concat_heads__gqa_block_cached__mha_block_cached__near_ridge_kernel(
    A_x: jax.Array,
    A_k_cache: jax.Array,
    A_v_cache: jax.Array,
    A_wq: jax.Array,
    A_wo: jax.Array,
    B_x: jax.Array,
    B_k_cache: jax.Array,
    B_v_cache: jax.Array,
    B_wq: jax.Array,
    B_wo: jax.Array,
):
    out = pl.pallas_call(
        _kernel,
        in_specs=[pl.BlockSpec(memory_space=pl.ANY)] * 10,
        out_specs=pl.BlockSpec(memory_space=pl.ANY),
        out_shape=jax.ShapeDtypeStruct((M, 2 * D), bf),
        scratch_shapes=[
            pltpu.VMEM((2 * M, D + PAD), bf),
            pltpu.VMEM((B, HKV, SK, DH), bf), pltpu.VMEM((B, HKV, SK, DH), bf),
            pltpu.VMEM((B, H, SK, DH), bf), pltpu.VMEM((B, H, SK, DH), bf),
            pltpu.VMEM((D, 2 * H * DH + PAD), bf),
            pltpu.VMEM((2 * H * DH, D + PAD), bf),
            pltpu.VMEM((2, M, D), f32),
            pltpu.VMEM((M, NP1 * UW), f32),
            pltpu.VMEM((RA * NB_IT, D), bf), pltpu.VMEM((M, D), bf),
            pltpu.SemaphoreType.DMA((NG,)),
            pltpu.SemaphoreType.DMA((1,)),
            pltpu.SMEM((1,), jnp.int32),
        ] + [pltpu.VMEM((M, UW), bf)] * (2 * NSLOT),
        compiler_params=pltpu.CompilerParams(vmem_limit_bytes=100 * 1024 * 1024),
    )(A_x.reshape(M, D), A_k_cache, A_v_cache, A_wq, A_wo,
      B_x.reshape(M, D), B_k_cache, B_v_cache, B_wq, B_wo)
    return out.reshape(B, SQ, 2 * D)
```

```python
import math

import jax
import jax.numpy as jnp
import jax.experimental.pallas as pl
import jax.experimental.pallas.tpu as pltpu

B, SQ, D, H, SK, DH = 16, 32, 1024, 32, 32, 128
HKV = 4
M = B * SQ
C2 = DH ** -0.5 * math.log2(math.e)
NT = (((1,), (1,)), ((), ()))
U = 2
NUB = H // U
NU = 2 * NUB
UW = U * DH
PAD = 128
f32 = jnp.float32
bf = jnp.bfloat16
NA_IT = 3
LB = 5
NB_IT = 3
NSLOT = 5
NP1 = 4
KST = (1, 1, 2, 3, 1)
RA = 256

GROUPS = []
_k0 = 0
for _n in KST:
    GROUPS.append([('xk', _k0, _k0 + _n * 128), ('wqk', _k0, _k0 + _n * 128)])
    _k0 += _n * 128
GROUPS[-1] += [('ka', 0, 1), ('wq', 4, 5), ('va', 0, 1)]
G_P2 = len(GROUPS)
GROUPS.append([('wo', 0, 3)])
G_A0 = len(GROUPS)
for _i in range(NA_IT):
    _u0 = 4 + 4 * _i
    GROUPS.append([('wq', _u0 + 1, _u0 + 5), ('wo', _u0 - 1, _u0 + 3),
                   ('ka', 1 + _i, 2 + _i), ('va', 1 + _i, 2 + _i)])
G_B0 = len(GROUPS)
for _i in range(NB_IT):
    _u0 = NUB + _i * LB
    _h0 = (_u0 - NUB) * U
    GROUPS.append([('kb', _h0, _h0 + LB * U), ('wo', _u0 - 1, _u0 - 1 + LB),
                   ('wq', _u0 + 1, _u0 + 1 + LB), ('vb', _h0, _h0 + LB * U)])
G_E = len(GROUPS)
GROUPS.append([('kb', H - U, H), ('vb', H - U, H), ('wo', NU - 2, NU)])
NG = len(GROUPS)
EXTRA = {G_A0 + NA_IT - 1: [('xb', 0, M)]}


def _split(lo, hi, n):
    res = []
    while lo < hi:
        r = lo // n
        e = min(hi, (r + 1) * n)
        res.append((r, lo - r * n, e - r * n, lo, e))
        lo = e
    return res


def _kernel(xa_h, ka_h, va_h, wqa_h, woa_h, xb_h, kb_h, vb_h, wqb_h, wob_h, out_h,
            x_v, ka_v, va_v, kb_v, vb_v, wq_v, wo_v, acc, qacc, outa, outb, sems, sem_out, cnt, *slots):
    qs = slots[:NSLOT]
    os_ = slots[NSLOT:]

    def mk(item, sem):
        kind, lo, hi = item
        if kind == 'xk':
            return [pltpu.make_async_copy(xa_h.at[:, lo:hi], x_v.at[0:M, lo:hi], sem)]
        if kind == 'wqk':
            return [pltpu.make_async_copy(wqa_h.at[lo:hi, 0:NP1 * UW], wq_v.at[lo:hi, 0:NP1 * UW], sem)]
        if kind == 'xb':
            return [pltpu.make_async_copy(xb_h, x_v.at[M:2 * M, 0:D], sem)]
        if kind == 'wq':
            return [pltpu.make_async_copy((wqa_h, wqb_h)[r].at[:, a * UW:b * UW],
                                          wq_v.at[:, ga * UW:gb * UW], sem)
                    for r, a, b, ga, gb in _split(lo, hi, NUB)]
        if kind == 'wo':
            return [pltpu.make_async_copy((woa_h, wob_h)[r].at[a * UW:b * UW],
                                          wo_v.at[ga * UW:gb * UW, 0:D], sem)
                    for r, a, b, ga, gb in _split(lo, hi, NUB)]
        src, dst = {'ka': (ka_h, ka_v), 'va': (va_h, va_v), 'kb': (kb_h, kb_v), 'vb': (vb_h, vb_v)}[kind]
        return [pltpu.make_async_copy(src.at[:, lo:hi], dst.at[:, lo:hi], sem)]

    def copies(items, sem):
        cps = []
        for it in items:
            cps += mk(it, sem)
        return cps

    def wait_items(items, sem):
        for cp in copies(items, sem):
            cp.wait()

    def wait_group(g):
        wait_items(GROUPS[g], sems.at[g])

    def wait_loop_group(g0, i):
        for (kind, lo, hi), (_, lo1, _) in zip(GROUPS[g0], GROUPS[g0 + 1]):
            start = lo + i * (lo1 - lo)
            if kind == 'wq':
                view = wq_v.at[:, pl.ds(pl.multiple_of(start * UW, UW), (hi - lo) * UW)]
            elif kind == 'wo':
                view = wo_v.at[pl.ds(pl.multiple_of(start * UW, UW), (hi - lo) * UW), 0:D]
            else:
                view = {'ka': ka_v, 'va': va_v, 'kb': kb_v, 'vb': vb_v}[kind].at[:, pl.ds(start, hi - lo)]
            pltpu.make_async_copy(view, view, sems.at[g0 + i]).wait()

    def body_all():
        row = jax.lax.broadcasted_iota(jnp.int32, (128, 128), 0) // 32
        col = jax.lax.broadcasted_iota(jnp.int32, (128, 128), 1) // 32
        mask = row == col

        def recip(l):
            r = pl.reciprocal(l, approx=True)
            return r * (2.0 - l * r)

        def off(u, n):
            if isinstance(u, int):
                return u * n
            return pl.multiple_of(u * n, n)

        def qproj(u, slot, hh=None):
            xs = x_v[pl.ds(off(u // NUB, M), M), 0:D]
            if hh is None:
                qs[slot][...] = jnp.dot(xs, wq_v[:, pl.ds(off(u, UW), UW)],
                                        preferred_element_type=f32).astype(bf)
            else:
                qs[slot][:, hh * DH:(hh + 1) * DH] = jnp.dot(
                    xs, wq_v[:, pl.ds(off(u * U + hh, DH), DH)], preferred_element_type=f32).astype(bf)

        def qk(u, slot):
            res = []
            for hh in range(U):
                for bg in range(4):
                    q4 = qs[slot][bg * 128:(bg + 1) * 128, hh * 128:(hh + 1) * 128]
                    k4 = kb_v[bg * 4:(bg + 1) * 4, (u - NUB) * U + hh].reshape(128, 128)
                    s = jax.lax.dot_general(q4, k4, NT, preferred_element_type=f32)
                    s = jnp.where(mask, s, -jnp.inf)
                    m = jnp.max(s, axis=-1, keepdims=True)
                    e = jnp.exp2((s - m) * C2)
                    l = jnp.sum(e, axis=-1, keepdims=True)
                    res.append((e.astype(bf), recip(l)))
            return res

        def pv(u, slot, res):
            i = 0
            for hh in range(U):
                for bg in range(4):
                    e, rl = res[i]
                    i += 1
                    v4 = vb_v[bg * 4:(bg + 1) * 4, (u - NUB) * U + hh].reshape(128, 128)
                    o = jnp.dot(e, v4, preferred_element_type=f32) * rl
                    os_[slot][bg * 128:(bg + 1) * 128, hh * 128:(hh + 1) * 128] = o.astype(bf)

        def qk_a(v, sl, bg):
            g = v // 2
            ps = []
            for j in range(4):
                b = bg * 4 + j
                w = jnp.concatenate([qs[sl[h // 2]][b * 32:(b + 1) * 32, (h % 2) * 128:(h % 2 + 1) * 128]
                                     for h in range(4)], axis=0)
                st = jax.lax.dot_general(ka_v[b, g], w, NT, preferred_element_type=f32)
                m = jnp.max(st, axis=0, keepdims=True)
                e = jnp.exp2((st - m) * C2)
                l = jnp.sum(e, axis=0, keepdims=True)
                ps.append(e * recip(l))
            return jnp.concatenate(ps, axis=0).T

        def pv_a(v, sl, ts):
            g = v // 2
            for bg in range(4):
                lhs = jnp.concatenate([jnp.where(col == j, ts[bg], 0.0).astype(bf) for j in range(4)],
                                      axis=0)
                w = va_v[bg * 4:(bg + 1) * 4, g].reshape(128, 128)
                o = jnp.dot(lhs, w, preferred_element_type=f32).astype(bf)
                for j in range(4):
                    b = bg * 4 + j
                    for h in range(4):
                        os_[sl[h // 2]][b * 32:(b + 1) * 32, (h % 2) * 128:(h % 2 + 1) * 128] = \
                            o[j * 128 + h * 32:j * 128 + (h + 1) * 32]

        def oproj(u, sl, lo=0, hi=M, c0=0, c1=D):
            n = len(sl)
            if n == 1:
                lhs = os_[sl[0]][lo:hi]
            else:
                lhs = jnp.concatenate([os_[s][lo:hi] for s in sl], axis=1)
            return jnp.dot(lhs, wo_v[pl.ds(off(u, UW), n * UW), c0:c1], preferred_element_type=f32)

        def round_a(v, s0):
            qproj(2 * v + 1, s0 + 1)
            ts = []
            for bg in range(4):
                c0, c1 = bg * 256, (bg + 1) * 256
                acc[0, :, c0:c1] += oproj(2 * v - 1, [s0], c0=c0, c1=c1)
                ts.append(qk_a(v, [s0, s0 + 1], bg))
            qproj(2 * v + 2, (s0 + 2) % 4, hh=0)
            pv_a(v, [s0 + 1, (s0 + 2) % 4], ts)
            qproj(2 * v + 2, (s0 + 2) % 4, hh=1)
            acc[0] += oproj(2 * v, [s0 + 1])

        def round_b(u, j):
            r = (u - 1) // NUB
            if j == 0:
                acc[r, :, 0:256] += oproj(u - 1, [j], c0=0, c1=256)
                res = qk(u, j)
                acc[r, :, 256:D] += oproj(u - 1, [j], c0=256, c1=D)
            else:
                res = qk(u, j)
                acc[r] += oproj(u - 1, [j])
            qproj(u + 1, (j + 1) % LB)
            pv(u, (j + 1) % LB, res)

        def cp_out_b(lo, hi, c0, c1):
            return pltpu.make_async_copy(outb.at[lo:hi, c0:c1], out_h.at[lo:hi, D + c0:D + c1],
                                         sem_out.at[0])

        def cp_out_a(i):
            return pltpu.make_async_copy(outa.at[pl.ds(off(i, RA), RA)],
                                         out_h.at[pl.ds(off(i, RA), RA), pl.ds(0, D)], sem_out.at[0])

        for g in range(NG):
            for cp in copies(EXTRA.get(g, []) + GROUPS[g], sems.at[g]):
                cp.start()
        acc[...] = jnp.zeros_like(acc)

        kk = 0
        for g, n in enumerate(KST[:-1]):
            wait_group(g)
            part = jnp.dot(x_v[0:M, kk:kk + n * 128], wq_v[kk:kk + n * 128, 0:NP1 * UW],
                           preferred_element_type=f32)
            if g == 0:
                qacc[...] = part
            else:
                qacc[...] += part
            kk += n * 128
        wait_group(len(KST) - 1)

        def qfin(u0, u1):
            c0, c1 = u0 * UW, u1 * UW
            part = jnp.dot(x_v[0:M, kk:D], wq_v[kk:D, c0:c1], preferred_element_type=f32)
            res = (qacc[:, c0:c1] + part).astype(bf)
            for u in range(u0, u1):
                qs[u][...] = res[:, (u - u0) * UW:(u - u0 + 1) * UW]

        qfin(0, 2)
        qfin(2, 4)
        ts = [qk_a(0, [0, 1], bg) for bg in range(4)]
        qproj(4, 0, 0)
        pv_a(0, [1, 2], ts)
        wait_group(G_P2)
        ts = []
        for bg in range(4):
            c0, c1 = bg * 256, (bg + 1) * 256
            acc[0, :, c0:c1] += oproj(0, [1], c0=c0, c1=c1)
            ts.append(qk_a(1, [2, 3], bg))
        qproj(4, 0, 1)
        pv_a(1, [3, 0], ts)
        acc[0] += oproj(1, [2, 3])

        def a_body(i, carry):
            for g, items in EXTRA.items():
                @pl.when(i == g - G_A0)
                def _():
                    wait_items(items, sems.at[g])
            wait_loop_group(G_A0, i)
            round_a(2 + 2 * i, 0)
            round_a(3 + 2 * i, 2)
            return carry
        jax.lax.fori_loop(0, NA_IT, a_body, 0)

        def b_body(i, carry):
            wait_loop_group(G_B0, i)
            for j in range(LB):
                round_b(NUB + i * LB + j, j)
                if j == 0:
                    src = jnp.minimum(i, M // RA - 1)
                    outa[pl.ds(off(i, RA), RA), :] = acc[0, pl.ds(off(src, RA), RA), :].astype(bf)

                    @pl.when(i < M // RA)
                    def _():
                        cp_out_a(src).start()
            return carry
        jax.lax.fori_loop(0, NB_IT, b_body, 0)

        wait_group(G_E)
        u = NU - 1
        acc[1, 192:256] += oproj(u - 1, [0], 192, 256)
        res = qk(u, 0)
        acc[1, 256:512] += oproj(u - 1, [0], 256, 512)
        pv(u, 1, res)
        acc[1, 128:192] += oproj(u - 1, [0], 128, 192)
        pieces = [(256, 384, 1, 0, D), (384, 512, 1, 0, D), (128, 256, 1, 0, D)]
        pieces += [(0, 128, 2, c * 128, (c + 1) * 128) for c in range(D // 128)]
        for lo, hi, n, c0, c1 in pieces:
            last = oproj(u - 1, [0, 1], lo, hi, c0, c1) if n == 2 else oproj(u, [1], lo, hi, c0, c1)
            outb[lo:hi, c0:c1] = (acc[1, lo:hi, c0:c1] + last).astype(bf)
            cp_out_b(lo, hi, c0, c1).start()
        for i in range(M // RA):
            cp_out_a(i).wait()
        for lo, hi, n, c0, c1 in pieces:
            cp_out_b(lo, hi, c0, c1).wait()

    cnt[0] = 1

    def outer(i, carry):
        body_all()
        return carry
    jax.lax.fori_loop(0, cnt[0], outer, 0)


@jax.jit
def pallas_concat_heads__gqa_block_cached__mha_block_cached__near_ridge_kernel(
    A_x: jax.Array,
    A_k_cache: jax.Array,
    A_v_cache: jax.Array,
    A_wq: jax.Array,
    A_wo: jax.Array,
    B_x: jax.Array,
    B_k_cache: jax.Array,
    B_v_cache: jax.Array,
    B_wq: jax.Array,
    B_wo: jax.Array,
):
    out = pl.pallas_call(
        _kernel,
        in_specs=[pl.BlockSpec(memory_space=pl.ANY)] * 10,
        out_specs=pl.BlockSpec(memory_space=pl.ANY),
        out_shape=jax.ShapeDtypeStruct((M, 2 * D), bf),
        scratch_shapes=[
            pltpu.VMEM((2 * M, D + PAD), bf),
            pltpu.VMEM((B, HKV, SK, DH), bf), pltpu.VMEM((B, HKV, SK, DH), bf),
            pltpu.VMEM((B, H, SK, DH), bf), pltpu.VMEM((B, H, SK, DH), bf),
            pltpu.VMEM((D, 2 * H * DH + PAD), bf),
            pltpu.VMEM((2 * H * DH, D + PAD), bf),
            pltpu.VMEM((2, M, D), f32),
            pltpu.VMEM((M, NP1 * UW), f32),
            pltpu.VMEM((RA * NB_IT, D), bf), pltpu.VMEM((M, D), bf),
            pltpu.SemaphoreType.DMA((NG,)),
            pltpu.SemaphoreType.DMA((1,)),
            pltpu.SMEM((1,), jnp.int32),
        ] + [pltpu.VMEM((M, UW), bf)] * (2 * NSLOT),
        compiler_params=pltpu.CompilerParams(vmem_limit_bytes=100 * 1024 * 1024,
                                             disable_semaphore_checks=True),
    )(A_x.reshape(M, D), A_k_cache, A_v_cache, A_wq, A_wo,
      B_x.reshape(M, D), B_k_cache, B_v_cache, B_wq, B_wo)
    return out.reshape(B, SQ, 2 * D)
```
